```python
import os as _os
_os.environ.setdefault("JAX_PLATFORMS", "cpu")
import jax
import jax.numpy as jnp

def _softmax(x, axis=-1):
    return jax.nn.softmax(x, axis=axis)
def _gelu(x):
    return jax.nn.gelu(x, approximate=True)
def _silu(x):
    return jax.nn.silu(x)
def _sigmoid(x):
    return jax.nn.sigmoid(x)
def _layernorm(x, axis=-1, eps=1e-5):
    m = jnp.mean(x, axis=axis, keepdims=True)
    v = jnp.var(x, axis=axis, keepdims=True)
    return (x - m) / jnp.sqrt(v + eps)
def _scatter_add(tgt, idx, src, axis=0):
    return tgt.at[idx].add(src)
def _segment_sum(src, seg, n):
    return jax.ops.segment_sum(src, seg, n)
class _Rng:
    def __init__(self, key):
        self._k = key
    def _next(self):
        self._k, sub = jax.random.split(self._k)
        return sub
    def normal(self, shape):
        return jax.random.normal(self._next(), shape, dtype=jnp.bfloat16)
    def randint(self, lo, hi, shape):
        return jax.random.randint(self._next(), shape, lo, hi, dtype=jnp.int32)
    def uniform(self, shape, lo=0.0, hi=1.0):
        return jax.random.uniform(self._next(), shape, jnp.bfloat16, lo, hi)
    def permutation(self, n):
        return jax.random.permutation(self._next(), n)


kernel_name = 'concat_heads__sliding_block_cached__sliding_block_cached__decode'

def setup_inputs():
    _rng = _Rng(jax.random.key(int.from_bytes(__import__("os").urandom(4), "little")))
    _w = (lambda a: (lambda t: t.astype(jnp.bfloat16) if jnp.issubdtype(t.dtype, jnp.floating) else t)(jnp.asarray(a)))
    def _A_setup():
        B, Sq, D = 4, 1, 576
        Hq, Hkv, Sk, Dh = 32, 16, 8192, 128
        assert Hq % Hkv == 0, (Hq, Hkv)
        return {
            "x": _w((lambda *s: _rng.normal(s) * 0.8)(B, Sq, D)),
            "k_cache": _w((lambda *s: _rng.normal(s) * 0.8)(B, Hkv, Sk, Dh)),
            "v_cache": _w((lambda *s: _rng.normal(s) * 0.05)(B, Hkv, Sk, Dh)),
            "wq": _w((lambda *s: _rng.normal(s) * 0.8)(D, Hq * Dh) * (D ** -0.5)),
            "wo": _w((lambda *s: _rng.normal(s) * 0.05)(Hq * Dh, D) * ((Hq * Dh) ** -0.5)),
        }
    _A_in = _A_setup()

    def _B_setup():
        B, Sq, D = 4, 1, 576
        Hq, Hkv, Sk, Dh = 32, 16, 8192, 128
        assert Hq % Hkv == 0, (Hq, Hkv)
        return {
            "x": _w((lambda *s: _rng.normal(s) * 0.8)(B, Sq, D)),
            "k_cache": _w((lambda *s: _rng.normal(s) * 0.8)(B, Hkv, Sk, Dh)),
            "v_cache": _w((lambda *s: _rng.normal(s) * 0.05)(B, Hkv, Sk, Dh)),
            "wq": _w((lambda *s: _rng.normal(s) * 0.8)(D, Hq * Dh) * (D ** -0.5)),
            "wo": _w((lambda *s: _rng.normal(s) * 0.05)(Hq * Dh, D) * ((Hq * Dh) ** -0.5)),
        }
    _B_in = _B_setup()

    return {
        "A_x": _A_in["x"],
        "A_k_cache": _A_in["k_cache"],
        "A_v_cache": _A_in["v_cache"],
        "A_wq": _A_in["wq"],
        "A_wo": _A_in["wo"],
        "B_x": _B_in["x"],
        "B_k_cache": _B_in["k_cache"],
        "B_v_cache": _B_in["v_cache"],
        "B_wq": _B_in["wq"],
        "B_wo": _B_in["wo"],
    }

def reference(A_x, A_k_cache, A_v_cache, A_wq, A_wo, B_x, B_k_cache, B_v_cache, B_wq, B_wo):
    def _A_ref(x, k_cache, v_cache, wq, wo):
        B, Sq, D = x.shape
        Hq, Dh = 32, 128
        Hkv, Sk = k_cache.shape[1], k_cache.shape[2]
        W = min(4096, max(256, Sk // 4))
        rep = Hq // Hkv
        q = (lambda x, *d: x.transpose(*d))((x @ wq).reshape(B, Sq, Hq, Dh), 0, 2, 1, 3)
        k = jnp.repeat(k_cache[:, :, Sk - W:, :], rep, axis=1)
        v = jnp.repeat(v_cache[:, :, Sk - W:, :], rep, axis=1)
        scores = jnp.einsum("bhqd,bhkd->bhqk", q, k) * (Dh ** -0.5)
        p = _softmax(scores, axis=-1)
        o = jnp.einsum("bhqk,bhkd->bhqd", p, v)
        return (lambda x, *d: x.transpose(*d))(o, 0, 2, 1, 3).reshape(B, Sq, Hq * Dh) @ wo

    def _B_ref(x, k_cache, v_cache, wq, wo):
        B, Sq, D = x.shape
        Hq, Dh = 32, 128
        Hkv, Sk = k_cache.shape[1], k_cache.shape[2]
        W = min(4096, max(256, Sk // 4))
        rep = Hq // Hkv
        q = (lambda x, *d: x.transpose(*d))((x @ wq).reshape(B, Sq, Hq, Dh), 0, 2, 1, 3)
        k = jnp.repeat(k_cache[:, :, Sk - W:, :], rep, axis=1)
        v = jnp.repeat(v_cache[:, :, Sk - W:, :], rep, axis=1)
        scores = jnp.einsum("bhqd,bhkd->bhqk", q, k) * (Dh ** -0.5)
        p = _softmax(scores, axis=-1)
        o = jnp.einsum("bhqk,bhkd->bhqd", p, v)
        return (lambda x, *d: x.transpose(*d))(o, 0, 2, 1, 3).reshape(B, Sq, Hq * Dh) @ wo

    a = _A_ref(A_x, A_k_cache, A_v_cache, A_wq, A_wo)
    b = _B_ref(B_x, B_k_cache, B_v_cache, B_wq, B_wo)
    return jnp.concatenate([a, b], axis=-1)
```

```python
import functools

import jax
import jax.numpy as jnp
from jax import lax
import jax.experimental.pallas as pl
import jax.experimental.pallas.tpu as pltpu

B, D, HQ, HKV, SK, DH = 4, 576, 32, 16, 8192, 128
W = min(4096, max(256, SK // 4))
OFF = SK - W
REP = HQ // HKV
HW = REP * DH
NT = (((1,), (1,)), ((), ()))
NN = (((1,), (0,)), ((), ()))


def make(GR=512, DR=32, WR=64, unroll=False, two_q=True, compute=True):
    NG = W // GR
    ND = GR // DR
    NTILE = (GR // 128) * B
    NWD = D // WR

    def kernel(xa, ka, va, wqa, woa, xb, kb, vb, wqb, wob, out_ref,
               xbuf, kbuf, vbuf, wqbuf, wobuf, sbuf, pbuf,
               xsem, ksem, vsem, wqsem, wosem):
        srcs = ((ka, va, wqa, woa), (kb, vb, wqb, wob))
        f32, bf16 = jnp.float32, jnp.bfloat16
        row = lax.broadcasted_iota(jnp.int32, (8, 128), 0)
        cnt = [0]

        def go(cp):
            cp.start(priority=(cnt[0] & 1) if two_q else 0)
            cnt[0] += 1

        def kv_dma(src, buf, sem, h, slot, g, i):
            r = pl.multiple_of(g * GR + i * DR, DR)
            return pltpu.make_async_copy(
                src.at[:, h, pl.ds(OFF + r, DR), :],
                buf.at[slot, :, pl.ds(r, DR), :], sem.at[slot, g])

        def kv_wait(buf, sem, slot, g):
            r = pl.multiple_of(g * GR, GR)
            v = buf.at[slot, :, pl.ds(r, GR), :]
            pltpu.make_async_copy(v, v, sem.at[slot, g]).wait()

        def w_dma(src, buf, sem, h, slot, i):
            c = pl.multiple_of(h * HW, HW)
            return pltpu.make_async_copy(
                src.at[pl.ds(i * WR, WR), pl.ds(c, HW)],
                buf.at[slot, pl.ds(i * WR, WR), :], sem.at[slot])

        def w_wait(buf, sem, slot):
            pltpu.make_async_copy(buf.at[slot], buf.at[slot], sem.at[slot]).wait()

        def loop(n, body, init):
            if unroll:
                c = init
                for g in range(n):
                    c = body(g, c)
                return c
            return lax.fori_loop(0, n, body, init)

        def step(br, slot, nxt, acc):
            ns = 1 - slot
            if nxt is not None:
                nk, nv, nwq, nwo = srcs[nxt[0]]
                nh = nxt[1]
            w_wait(wqbuf, wqsem, slot)
            if nxt is not None:
                for i in range(NWD):
                    go(w_dma(nwq, wqbuf, wqsem, nh, ns, i))
            qq = lax.dot_general(xbuf[br].astype(bf16), wqbuf[slot], NN, preferred_element_type=f32)
            q8 = jnp.where(row < B, qq[:, :DH], qq[:, DH:]).astype(bf16)

            def kgrp(g, m):
                kv_wait(kbuf, ksem, slot, g)
                c0 = cnt[0]
                n = 0
                for t in range(GR // 128):
                    r = pl.multiple_of(g * GR + t * 128, 128)
                    s = None
                    for b in range(B):
                        if nxt is not None:
                            while n * NTILE < (t * B + b + 1) * ND:
                                go(kv_dma(nk, kbuf, ksem, nh, ns, g, n))
                                n += 1
                        if compute:
                            sb = lax.dot_general(q8, kbuf[slot, b, pl.ds(r, 128), :], NT,
                                                 preferred_element_type=f32)
                            s = sb if s is None else jnp.where((row & (B - 1)) == b, sb, s)
                    if compute:
                        s = s * (DH ** -0.5)
                        sbuf[g * (GR // 128) + t] = s
                        m = jnp.maximum(m, s)
                assert (cnt[0] - c0) % 2 == 0
                return m
            m = loop(NG, kgrp, jnp.full((8, 128), -jnp.inf, f32))
            m = jnp.max(m, axis=1, keepdims=True)
            if nxt is not None:
                for i in range(NWD):
                    go(w_dma(nwo, wobuf, wosem, nh, ns, i))

            def vgrp(g, c):
                l, os = c
                os = list(os)
                kv_wait(vbuf, vsem, slot, g)
                n = 0
                for t in range(GR // 128):
                    r = pl.multiple_of(g * GR + t * 128, 128)
                    if compute:
                        p = jnp.exp(sbuf[g * (GR // 128) + t] - m)
                        l = l + p
                        pb = p.astype(bf16)
                    for b in range(B):
                        if nxt is not None:
                            while n * NTILE < (t * B + b + 1) * ND:
                                go(kv_dma(nv, vbuf, vsem, nh, ns, g, n))
                                n += 1
                        if compute:
                            os[b] = os[b] + lax.dot_general(pb, vbuf[slot, b, pl.ds(r, 128), :], NN,
                                                            preferred_element_type=f32)
                return l, tuple(os)
            z = jnp.zeros((8, 128), f32)
            l, os = loop(NG, vgrp, (z, (z,) * B))
            o = os[0]
            for b in range(1, B):
                o = jnp.where((row & (B - 1)) == b, os[b], o)
            o = (o / jnp.sum(l, axis=1, keepdims=True)).astype(bf16)
            w_wait(wobuf, wosem, slot)
            r0 = lax.dot_general(o, wobuf[slot, :, :DH], NT, preferred_element_type=f32)
            r1 = lax.dot_general(o, wobuf[slot, :, DH:], NT, preferred_element_type=f32)
            rowd = lax.broadcasted_iota(jnp.int32, (8, D), 0)
            return acc + jnp.where(rowd < B, r0, r1)

        xc = [pltpu.make_async_copy(xa, pbuf.at[0], xsem.at[0]),
              pltpu.make_async_copy(xb, pbuf.at[1], xsem.at[1])]
        for i in range(NWD):
            go(w_dma(wqa, wqbuf, wqsem, 0, 0, i))
        for c in xc:
            c.start()

        def pro_k(g, c):
            for i in range(ND):
                go(kv_dma(ka, kbuf, ksem, 0, 0, g, i))
            return c
        lax.fori_loop(0, NG, pro_k, 0)
        for i in range(NWD):
            go(w_dma(woa, wobuf, wosem, 0, 0, i))

        def pro_v(g, c):
            for i in range(ND):
                go(kv_dma(va, vbuf, vsem, 0, 0, g, i))
            return c
        lax.fori_loop(0, NG, pro_v, 0)
        for i, c in enumerate(xc):
            c.wait()
            xv = pbuf[i].astype(f32)
            xbuf[i, 0:B, :] = xv
            xbuf[i, B:2 * B, :] = xv

        def pair(h, accs):
            a = step(0, 0, (1, h), accs[0])
            b = step(1, 1, (0, h + 1), accs[1])
            return a, b
        z = jnp.zeros((8, D), f32)
        accs = lax.fori_loop(0, HKV - 1, pair, (z, z))
        a = step(0, 0, (1, HKV - 1), accs[0])
        b = step(1, 1, None, accs[1])
        out_ref[:, 0:D] = (a[0:B] + a[B:]).astype(out_ref.dtype)
        out_ref[:, D:] = (b[0:B] + b[B:]).astype(out_ref.dtype)

    def fn(A_x, A_k_cache, A_v_cache, A_wq, A_wo, B_x, B_k_cache, B_v_cache, B_wq, B_wo):
        hbm = pl.BlockSpec(memory_space=pl.ANY)
        out = pl.pallas_call(
            kernel,
            in_specs=[hbm] * 10,
            out_specs=pl.BlockSpec(memory_space=pltpu.VMEM),
            out_shape=jax.ShapeDtypeStruct((B, 2 * D), A_x.dtype),
            scratch_shapes=[
                pltpu.VMEM((2, 2 * B, D), jnp.float32),
                pltpu.VMEM((2, B, W, DH), jnp.bfloat16),
                pltpu.VMEM((2, B, W, DH), jnp.bfloat16),
                pltpu.VMEM((2, D, HW), jnp.bfloat16),
                pltpu.VMEM((2, D, HW), jnp.bfloat16),
                pltpu.VMEM((W // 128, 8, 128), jnp.float32),
                pltpu.VMEM((2, B, D), jnp.bfloat16),
                pltpu.SemaphoreType.DMA((2,)),
                pltpu.SemaphoreType.DMA((2, NG)),
                pltpu.SemaphoreType.DMA((2, NG)),
                pltpu.SemaphoreType.DMA((2,)),
                pltpu.SemaphoreType.DMA((2,)),
            ],
            compiler_params=pltpu.CompilerParams(vmem_limit_bytes=32 * 1024 * 1024),
        )(A_x.reshape(B, D), A_k_cache, A_v_cache, A_wq, A_wo.T,
          B_x.reshape(B, D), B_k_cache, B_v_cache, B_wq, B_wo.T)
        return out.reshape(B, 1, 2 * D)
    return fn


@jax.jit
def pallas_concat_heads__sliding_block_cached__sliding_block_cached__decode_kernel(
    A_x, A_k_cache, A_v_cache, A_wq, A_wo, B_x, B_k_cache, B_v_cache, B_wq, B_wo):
    return make()(A_x, A_k_cache, A_v_cache, A_wq, A_wo, B_x, B_k_cache, B_v_cache, B_wq, B_wo)
```

```python
import jax
import jax.numpy as jnp
from jax import lax
import jax.experimental.pallas as pl
import jax.experimental.pallas.tpu as pltpu

B, D, HQ, HKV, SK, DH = 4, 576, 32, 16, 8192, 128
WIN = min(4096, max(256, SK // 4))
REP = HQ // HKV
ROWS = REP * B
HP = 2
NSTEP = HKV // HP
NATT = 2 * HP
PIECES = HP * REP
PCOLS = PIECES * DH
T = 128
NGRP = WIN // T
LAG = NGRP // 2
KV_ROWS = 64
SLABS, SLAB = 4, D // 4
W_ROWS, W_COLS = 8, 1024
K, V = 0, 1
WQ, WO = 0, 1
NN = (((1,), (0,)), ((), ()))
NT = (((1,), (1,)), ((), ()))

assert ROWS == 8 and B == 4 and PIECES == 4 and 2 * PIECES == LAG == 8


def _dot(a, b, dims):
    return lax.dot_general(a.astype(jnp.bfloat16), b, dims,
                           preferred_element_type=jnp.float32)


def _attend(xa, ka, va, wqa, woa, xb, kb, vb, wqb, wob, out_copy,
            out_buf, x_in, x_buf, kv_buf, w_buf, q_buf, s_buf, o_buf, acc, sem):
    kv_hbm = ((ka, kb), (va, vb))
    w_hbm = ((wqa, wqb), (woa, wob))
    w_sem = (sem.at[0], sem.at[LAG])
    row = lax.broadcasted_iota(jnp.int32, (ROWS, T), 0)
    row_d = lax.broadcasted_iota(jnp.int32, (ROWS, D), 0)
    tiles = [(br, h, b) for br in range(2) for h in range(HP) for b in range(B)]

    def start(copies):
        for n, c in enumerate(copies):
            c.start(priority=n % 2)

    def wait_filled(buf, s):
        pltpu.make_async_copy(buf, buf, s).wait()

    def kv_copies(kind, step, t):
        return [
            pltpu.make_async_copy(
                kv_hbm[kind][br].at[
                    b, pl.ds(step * HP, HP),
                    pl.ds(pl.multiple_of(SK - WIN + t * T + r, KV_ROWS), KV_ROWS), :],
                kv_buf.at[kind * NGRP + t, br, b, :, pl.ds(r, KV_ROWS), :],
                sem.at[t & (LAG - 1)])
            for r in range(0, T, KV_ROWS) for br in range(2) for b in range(B)]

    def wait_kv(kind, t):
        wait_filled(kv_buf.at[kind * NGRP + t], sem.at[t & (LAG - 1)])

    def load_weight(kind, ncols):
        def body(i, carry):
            copies = []
            for r in (0, W_ROWS):
                rows = pl.ds(pl.multiple_of(i * 2 * W_ROWS + r, W_ROWS), W_ROWS)
                for c in range(0, ncols, W_COLS):
                    nc = min(W_COLS, ncols - c)
                    ns = 2 * W_COLS // nc
                    for br in range(2):
                        for s in range(0, SLABS, ns):
                            idx = (pl.ds(s, ns), rows, pl.ds(c, nc))
                            copies.append(pltpu.make_async_copy(
                                w_hbm[kind][br].at[idx],
                                w_buf.at[(kind, br) + idx], w_sem[kind]))
            start(copies)
            return carry
        lax.fori_loop(0, SLAB // (2 * W_ROWS), body, 0)

    def last_wo_copies(br, slot):
        cols = pl.ds(pl.multiple_of(
            (NSTEP - 1) * PCOLS + (slot & (PIECES - 1)) * DH, DH), DH)
        return [pltpu.make_async_copy(w_hbm[WO][br].at[s, :, cols],
                                      w_buf.at[WO, br, s, :, cols], sem.at[slot])
                for s in range(SLABS)]

    def batched_dots(lhs, g, dims, copies):
        out = [None] * NATT
        n = 0
        for i, (br, h, b) in enumerate(tiles):
            while n * len(tiles) < (i + 1) * len(copies):
                copies[n].start(priority=n % 2)
                n += 1
            j = br * HP + h
            r = _dot(lhs[j], kv_buf[g, br, b, h], dims)
            out[j] = r if b == 0 else jnp.where((row & (B - 1)) == b, r, out[j])
        return out

    def weight_piece(kind, step, piece):
        br = piece >> 2
        c = pl.multiple_of(step * PCOLS + (piece & (PIECES - 1)) * DH, DH)
        return br, w_buf[kind, br, :, :, pl.ds(c, DH)].reshape(D, DH)

    def q_piece(step, piece):
        br, w = weight_piece(WQ, step, piece)
        q_buf[piece] = _dot(x_buf[br], w, NN)

    def out_piece(step, piece, o, live=True):
        br, w = weight_piece(WO, step, piece)
        keep = ((row_d >> 2) == (piece & 1)) & live
        return br, jnp.where(keep, _dot(o, w, NT), 0.0)

    def score_loop(lo, hi, q, m, prefetch, extra=None):
        def body(t, m):
            wait_kv(K, t)
            s = batched_dots(q, t, NT, prefetch(t))
            if extra is not None:
                extra(t)
            s = [x * (DH ** -0.5) for x in s]
            for j in range(NATT):
                s_buf[t, j] = s[j]
            return [jnp.maximum(a, x) for a, x in zip(m, s)]
        return lax.fori_loop(lo, hi, body, m)

    def value_loop(lo, hi, m, carry, prefetch, extra=None):
        def body(t, carry):
            wait_kv(V, t)
            p = [jnp.exp(s_buf[t, j] - m[j]) for j in range(NATT)]
            o = batched_dots(p, NGRP + t, NN, prefetch(t))
            if extra is not None:
                extra(t)
            return ([a + x for a, x in zip(carry[0], p)],
                    [a + x for a, x in zip(carry[1], o)])
        return lax.fori_loop(lo, hi, body, carry)

    def normalized(carry):
        return [o / jnp.sum(l, axis=1, keepdims=True) for l, o in zip(*carry)]

    x_copies = [pltpu.make_async_copy(x, x_in.at[i], sem.at[1 + i])
                for i, x in enumerate((xa, xb))]
    early_cols = HQ * DH - PCOLS
    load_weight(WQ, HQ * DH)
    start(x_copies)
    load_weight(WO, early_cols)
    for i, c in enumerate(x_copies):
        c.wait()
        x = x_in[i].astype(jnp.float32)
        for r in range(REP):
            x_buf[i, r * B:(r + 1) * B, :] = x
    acc[...] = jnp.zeros(acc.shape, acc.dtype)
    o_buf[...] = jnp.zeros(o_buf.shape, o_buf.dtype)
    wait_filled(w_buf.at[WQ], w_sem[WQ])

    def first_keys(t, carry):
        start(kv_copies(K, 0, t))
        q_piece(0, t)
        return carry
    lax.fori_loop(0, LAG, first_keys, 0)
    wait_filled(w_buf.at[WO, :, :, :, pl.ds(0, early_cols)], w_sem[WO])

    zeros = [jnp.zeros((ROWS, T), jnp.float32)] * NATT

    def step(s, _):
        q = [jnp.where(row < B, q_buf[REP * j], q_buf[REP * j + 1]).astype(jnp.bfloat16)
             for j in range(NATT)]

        def previous_out(t):
            br, r = out_piece(jnp.maximum(s - 1, 0), t, o_buf[t >> 1], s > 0)
            acc[br] += r

        m = [jnp.full((ROWS, T), -jnp.inf, jnp.float32)] * NATT
        m = score_loop(0, LAG, q, m, lambda t: kv_copies(K, s, t + LAG), previous_out)
        m = score_loop(LAG, NGRP, q, m, lambda t: kv_copies(V, s, t - LAG))
        m = [jnp.broadcast_to(jnp.max(x, axis=1, keepdims=True), (ROWS, T)) for x in m]
        half = value_loop(0, LAG, m, (zeros, zeros), lambda t: kv_copies(V, s, t + LAG),
                          lambda t: q_piece(jnp.minimum(s + 1, NSTEP - 1), t))

        @pl.when(s < NSTEP - 1)
        def _next():
            full = value_loop(LAG, NGRP, m, half, lambda t: kv_copies(K, s + 1, t - LAG))
            for j, o in enumerate(normalized(full)):
                o_buf[j] = o

        return m, half

    m, carry = lax.fori_loop(0, NSTEP, step, (zeros, (zeros, zeros)))

    branches = (1, 0)
    for n, br in enumerate(branches):
        lo = LAG + n * PIECES
        carry = value_loop(lo, lo + PIECES, m, carry,
                           lambda t, br=br: last_wo_copies(br, t - LAG))
    o = normalized(carry)
    for n, br in enumerate(branches):
        res = acc[br]
        for h in range(HP):
            for r in range(REP):
                for c in last_wo_copies(br, n * PIECES + h * REP + r):
                    c.wait()
            for r in range(REP):
                piece = br * PIECES + h * REP + r
                res = res + out_piece(NSTEP - 1, piece, o[br * HP + h])[1]
        out_buf[:, br * D:(br + 1) * D] = (res[:B] + res[B:]).astype(out_buf.dtype)
    out_copy.start()


def _kernel(*refs):
    ins, out_hbm, scratch, out_sem = refs[:10], refs[10], refs[11:-1], refs[-1]
    out_copy = pltpu.make_async_copy(scratch[0], out_hbm, out_sem.at[0])
    pl.run_scoped(lambda sem: _attend(*ins, out_copy, *scratch, sem),
                  pltpu.SemaphoreType.DMA((LAG + 1,)))
    out_copy.wait()


@jax.jit
def pallas_concat_heads__sliding_block_cached__sliding_block_cached__decode_kernel(
    A_x: jax.Array,
    A_k_cache: jax.Array,
    A_v_cache: jax.Array,
    A_wq: jax.Array,
    A_wo: jax.Array,
    B_x: jax.Array,
    B_k_cache: jax.Array,
    B_v_cache: jax.Array,
    B_wq: jax.Array,
    B_wo: jax.Array,
):
    assert A_k_cache.shape == B_k_cache.shape == (B, HKV, SK, DH)
    hbm = pl.BlockSpec(memory_space=pl.ANY)
    w_shape = (SLABS, SLAB, HQ * DH)
    out = pl.pallas_call(
        _kernel,
        in_specs=[hbm] * 10,
        out_specs=hbm,
        out_shape=jax.ShapeDtypeStruct((B, 2 * D), jnp.bfloat16),
        scratch_shapes=[
            pltpu.VMEM((B, 2 * D), jnp.bfloat16),
            pltpu.VMEM((2, B, D), jnp.bfloat16),
            pltpu.VMEM((2, ROWS, D), jnp.float32),
            pltpu.VMEM((2 * NGRP, 2, B, HP, T, DH), jnp.bfloat16),
            pltpu.VMEM((2, 2) + w_shape, jnp.bfloat16),
            pltpu.VMEM((2 * PIECES, ROWS, DH), jnp.float32),
            pltpu.VMEM((NGRP, NATT, ROWS, T), jnp.float32),
            pltpu.VMEM((NATT, ROWS, DH), jnp.float32),
            pltpu.VMEM((2, ROWS, D), jnp.float32),
            pltpu.SemaphoreType.DMA((1,)),
        ],
        compiler_params=pltpu.CompilerParams(vmem_limit_bytes=48 * 1024 * 1024),
    )(A_x.reshape(B, D), A_k_cache, A_v_cache,
      A_wq.reshape(w_shape), A_wo.T.reshape(w_shape),
      B_x.reshape(B, D), B_k_cache, B_v_cache,
      B_wq.reshape(w_shape), B_wo.T.reshape(w_shape))
    return out.reshape(B, 1, 2 * D)
```
